```python
import jax
import jax.numpy as jnp

def _softmax(x, axis=-1):
    return jax.nn.softmax(x, axis=axis)
def _gelu(x):
    return jax.nn.gelu(x, approximate=True)
def _silu(x):
    return jax.nn.silu(x)
def _sigmoid(x):
    return jax.nn.sigmoid(x)
def _layernorm(x, axis=-1, eps=1e-5):
    m = jnp.mean(x, axis=axis, keepdims=True)
    v = jnp.var(x, axis=axis, keepdims=True)
    return (x - m) / jnp.sqrt(v + eps)
def _scatter_add(tgt, idx, src, axis=0):
    return tgt.at[idx].add(src)
def _segment_sum(src, seg, n):
    return jax.ops.segment_sum(src, seg, n)
class _Rng:
    def __init__(self, key):
        self._k = key
    def _next(self):
        self._k, sub = jax.random.split(self._k)
        return sub
    def normal(self, shape):
        return jax.random.normal(self._next(), shape, dtype=jnp.bfloat16)
    def randint(self, lo, hi, shape):
        return jax.random.randint(self._next(), shape, lo, hi, dtype=jnp.int32)
    def uniform(self, shape, lo=0.0, hi=1.0):
        return jax.random.uniform(self._next(), shape, jnp.bfloat16, lo, hi)
    def permutation(self, n):
        return jax.random.permutation(self._next(), n)


kernel_name = 'standalone__structured_sparse_n_m__ragged'

def setup_inputs():
    _rng = _Rng(jax.random.key(int.from_bytes(__import__("os").urandom(4), "little")))
    _w = (lambda a: (lambda t: t.astype(jnp.bfloat16) if jnp.issubdtype(t.dtype, jnp.floating) else t)(jnp.asarray(a)))
    B, S, D = 16, 4096, 576
    assert D % 4 == 0, "d_model must be divisible by M=4 for 2:4 sparsity"
    return {
        "x": _w((lambda *s: _rng.normal(s) * 0.05)(B, S, D)),
        "w": _w((lambda *s: _rng.normal(s) * 0.05)(D, D)),
        "b": _w((lambda *s: _rng.normal(s) * 0.05)(D)),
    }

def reference(x, w, b):
    B, S, D = x.shape
    N, M = 2, 4
    G = D // M
    wg = w.reshape(G, M, D)
    mag = jnp.abs(wg)
    order = jnp.argsort(mag, 1)
    thr = jnp.take_along_axis(mag, order[:, M - N:M - N + 1, :], 1)
    mask = (lambda x, dt: x.astype(dt))(mag >= thr, w.dtype)
    wp = (wg * mask).reshape(D, D)
    return jnp.einsum("bsd,df->bsf", x, wp) + b
```

```python
import jax
import jax.numpy as jnp
from jax import lax
import jax.experimental.pallas as pl
import jax.experimental.pallas.tpu as pltpu

F32, BF16, I32 = jnp.float32, jnp.bfloat16, jnp.int32

H = 144
STEP = 512
NX = 9
IN_SPLIT = (512, 512, 1024, 2048)
FIRST_WRITE = 65
WRITES = 16


def _prune_packed(u):
    mate = lax.broadcasted_iota(I32, u.shape, 0) ^ 1
    lo = pltpu.bitcast((u << 16) & 0x7FFFFFFF, F32)
    hi = pltpu.bitcast(u & 0x7FFF0000, F32)
    big, small = jnp.maximum(lo, hi), jnp.minimum(lo, hi)
    nbig = jnp.take_along_axis(big, mate, axis=0, mode="promise_in_bounds")
    nsmall = jnp.take_along_axis(small, mate, axis=0, mode="promise_in_bounds")
    thr = jnp.maximum(jnp.minimum(big, nbig), jnp.maximum(small, nsmall))
    return u & (jnp.where(lo < thr, 0, 0xFFFF) | jnp.where(hi < thr, 0, -65536))


def _prune_rows(w_bf16):
    u = pltpu.bitcast(w_bf16, I32)
    return [_prune_packed(u[8 * i:8 * i + 8]) for i in range(u.shape[0] // 8)]


def _lhs(a11, a12, a21, a22):
    return [a11 + a22, a21 + a22, a11, a22, a11 + a12, a21 - a11, a12 - a22]


_RHS = [(0, 3), (0, None), (1, 3), (2, 0), (3, None), (1, 0), (2, 3)]


def _rhs(*b):
    return [b[p] if q is None else b[p] - b[q] for p, q in _RHS]


def _combine(m):
    return [(m[0] + m[3]) + (m[4] + m[6]), m[2] + m[4], m[1] + m[3],
            (m[1] - m[0]) + (m[2] + m[5])]


_T_OF_P = [None, 1, 3, 2, 4]


def _prepare_weights(wbuf, bbuf, wt_ref, bias_ref):
    def transposed(parts):
        return pltpu.bitcast(jnp.concatenate(parts, axis=0), BF16).T.astype(F32)

    kt = [transposed(_prune_rows(wbuf[128 * i:128 * (i + 1), :])) for i in range(4)]
    tail = _prune_rows(wbuf[512:576, :])
    kt.append(transposed(tail + tail))
    low = lax.broadcasted_iota(I32, (H, 128), 1) < 64

    def quarter(t, i):
        return kt[t][H * i:H * (i + 1)]

    def put(n, v):
        wt_ref[n] = pltpu.bitcast(v.astype(BF16), I32)

    full = [_lhs(quarter(0, i), quarter(1, i), quarter(0, i + 2), quarter(1, i + 2)) for i in range(2)]
    half = [_lhs(quarter(2, i), quarter(3, i), quarter(2, i + 2), quarter(3, i + 2)) for i in range(2)]
    for c in range(7):
        blocks = []
        for i in range(2):
            if c == 0:
                mixed = jnp.where(low, half[i][0], 0.0)
            elif c >= 5:
                mixed = jnp.where(low, half[i][c], quarter(4, i + 2 if c == 5 else i))
            elif _T_OF_P[c] == c:
                mixed = half[i][c]
            else:
                mixed = jnp.where(low, half[i][c], half[i][_T_OF_P[c]])
            blocks += [full[i][c], mixed]
        for n, v in enumerate(_lhs(*blocks)):
            put(7 * c + n, v)
    for i in range(2):
        put(49 + i, jnp.where(low, 0.0, half[i][0]))
        put(51 + i, jnp.where(low, quarter(4, i + 2), half[i][5]))
        put(53 + i, jnp.where(low, quarter(4, i), half[i][6]))
    bias = bbuf[...].reshape(1, 576).astype(F32)
    bias_ref[...] = jnp.broadcast_to(bias, (128, 576)).T


def _step(load_x, store, wt_ref, bias_ref):
    zeros = jnp.zeros((64, 128), F32)

    def cat(*parts):
        return jnp.concatenate(parts, axis=0)

    def level1(which, src, rows):
        p, q = _RHS[which]
        v = load_x(src[p][0], rows, src[p][1])
        return v if q is None else v - load_x(src[q][0], rows, src[q][1])

    def s_rhs(which, r1, r2, rows, j):
        return level1(which, [(r1, j), (r1, j + 2), (r2, j), (r2, j + 2)], rows)

    def t_rhs(which, j):
        return level1(which, [(320, j + 2), (320, j), (448, j + 2), (448, j)], 64)

    def dot(n, rhs):
        return jnp.dot(pltpu.bitcast(wt_ref[n], BF16), rhs, preferred_element_type=F32)

    def p_block(c, bias_quarter=None):
        top = [s_rhs(c, 0, 128, 128, j) for j in range(2)]
        lo = _rhs(top[0][:64], top[1][:64], *[s_rhs(c, 256, 384, 64, j) for j in range(2)])
        t0, t1 = top[0][64:], top[1][64:]
        if c == 0:
            hi = [t0, t0, t1, zeros, zeros, t1 - t0, zeros]
        elif c >= 5:
            hi = _rhs(t0, t1, *[load_x(512, 64, j + 2 if c == 5 else j) for j in range(2)])
        else:
            hi = _rhs(t0, t1, *[t_rhs(_T_OF_P[c], j) for j in range(2)])
        rhs = [cat(u, v).astype(BF16) for u, v in zip(lo, hi)]
        m = [dot(7 * c + n, rhs[n]) for n in range(7)]
        if bias_quarter is not None:
            m[4] = m[4] + bias_ref[pl.ds(H * bias_quarter, H), :]
            m[1] = m[1] + bias_ref[pl.ds(H * (bias_quarter + 1), H), :]
        return _combine(m)

    def q_block(q):
        out = [None] * 4
        for j in range(2):
            if q == 0:
                rhs = cat(zeros, t_rhs(0, j))
            else:
                rhs = cat(load_x(512, 64, j if q == 1 else j + 2), t_rhs(4 + q, j))
            rhs = rhs.astype(BF16)
            for i in range(2):
                out[2 * i + j] = dot(49 + 2 * q + i, rhs)
        return out

    def put(row_half, token_half, vals):
        for i in range(2):
            for j in range(2):
                store(2 * row_half + i, 2 * token_half + j, vals[2 * i + j].astype(BF16))

    def add(a, b):
        return [u + v for u, v in zip(a, b)]

    def sub(a, b):
        return [u - v for u, v in zip(a, b)]

    p0 = p_block(0)
    c11 = add(p0, p_block(6))
    p3 = p_block(3)
    p4 = p_block(4, 0)
    put(0, 0, add(c11, add(p3, p4)))
    p2 = p_block(2)
    p1 = p_block(1, 2)
    put(1, 1, add(sub(p1, p0), add(p2, p_block(5))))
    q0 = q_block(0)
    put(1, 0, add(add(p1, p3), sub(q_block(1), q0)))
    put(0, 1, add(add(p2, p4), add(q_block(2), q0)))


def _kernel(x_hbm, w_hbm, b_hbm, o_hbm, xbuf, obuf, wbuf, bbuf, wt_ref, bias_ref,
            isem, osem, psem):
    NB, _, S = x_hbm.shape
    steps = S // STEP
    offsets = [sum(IN_SPLIT[:j]) for j in range(len(IN_SPLIT))]
    n_in = len(IN_SPLIT)

    def icopy(b, slot, j):
        cols = pl.ds(offsets[j], IN_SPLIT[j])
        return pltpu.make_async_copy(
            x_hbm.at[b, :, cols], xbuf.at[slot, :, cols], isem.at[slot * n_in + j])

    def ocopy(d):
        b, q = d >> 6, d & 63
        last = b == NB - 1
        band = jnp.where(last, q & 7, q >> 3)
        cols = pl.ds(pl.multiple_of(jnp.where(last, q >> 3, q & 7) * STEP, STEP), STEP)
        return pltpu.make_async_copy(
            obuf.at[b, :, band, :, cols], o_hbm.at[b, :, band, :, cols], osem)

    wcopy = pltpu.make_async_copy(w_hbm, wbuf, psem.at[0])
    bcopy = pltpu.make_async_copy(b_hbm, bbuf, psem.at[1])
    wcopy.start()
    bcopy.start()
    for b in range(NX):
        for j in range(n_in):
            icopy(b, b, j).start()
    wcopy.wait()
    bcopy.wait()
    _prepare_weights(wbuf, bbuf, wt_ref, bias_ref)

    def body(b, carry):
        slot = jnp.where(b >= NX, b - NX, b)
        for s in range(steps):
            col = s * STEP
            if col in offsets:
                icopy(b, slot, offsets.index(col)).wait()
            g = b * steps + s
            for e in range(WRITES):
                copy = ocopy(jnp.maximum(g - FIRST_WRITE, 0) * WRITES + e)
                pl.when(g >= FIRST_WRITE)(copy.start)

            def load_x(row, rows, tile):
                return xbuf[slot, pl.ds(row, rows), pl.ds(col + tile * 128, 128)].astype(F32)

            def store(quarter, tile, v):
                for k in range(H // 8):
                    band = quarter * (H // 8) + k
                    obuf[b, band // 8, band % 8, :, pl.ds(col + tile * 128, 128)] = v[8 * k:8 * k + 8]

            _step(load_x, store, wt_ref, bias_ref)
        for j in range(n_in):
            copy = icopy(jnp.minimum(b + NX, NB - 1), slot, j)
            pl.when(b + NX < NB)(copy.start)
        return carry

    lax.fori_loop(0, NB, body, 0)
    for d in range((NB * steps - FIRST_WRITE) * WRITES, NB * 64):
        ocopy(d).start()
    pltpu.make_async_copy(obuf, o_hbm, osem).wait()


@jax.jit
def pallas_standalone__structured_sparse_n_m__ragged_kernel(
    x: jax.Array,
    w: jax.Array,
    b: jax.Array,
):
    B, S, D = x.shape
    assert (S, D) == (4096, 576) and w.shape == (D, D) and B >= NX
    out = pl.pallas_call(
        _kernel,
        in_specs=[pl.BlockSpec(memory_space=pl.ANY)] * 3,
        out_specs=pl.BlockSpec(memory_space=pl.ANY),
        out_shape=jax.ShapeDtypeStruct((B, 9, 8, 8, S), x.dtype),
        scratch_shapes=[
            pltpu.VMEM((NX, D, S), x.dtype),
            pltpu.VMEM((B, 9, 8, 8, S), x.dtype),
            pltpu.VMEM((D, D), w.dtype),
            pltpu.VMEM((D,), b.dtype),
            pltpu.VMEM((55, H // 2, 128), I32),
            pltpu.VMEM((D, 128), F32),
            pltpu.SemaphoreType.DMA((NX * len(IN_SPLIT),)),
            pltpu.SemaphoreType.DMA(()),
            pltpu.SemaphoreType.DMA((2,)),
        ],
        compiler_params=pltpu.CompilerParams(
            vmem_limit_bytes=127 * 1024 * 1024,
            disable_bounds_checks=True,
            flags={"XLA_TPU_RESCHEDULE_DMA_DONES": True},
        ),
    )(jnp.transpose(x, (0, 2, 1)), w, b)
    return jnp.transpose(out.reshape(B, D, S), (0, 2, 1))
```

```python
import functools

import jax
import jax.numpy as jnp
from jax import lax
import jax.experimental.pallas as pl
import jax.experimental.pallas.tpu as pltpu

F32, BF16, I32 = jnp.float32, jnp.bfloat16, jnp.int32

D = 576
H = D // 4
SLAB = 16


def _prune_packed(u):
    mate = lax.broadcasted_iota(I32, u.shape, 0) ^ 1
    lo = pltpu.bitcast((u << 16) & 0x7FFFFFFF, F32)
    hi = pltpu.bitcast(u & 0x7FFF0000, F32)
    big, small = jnp.maximum(lo, hi), jnp.minimum(lo, hi)
    nbig = jnp.take_along_axis(big, mate, axis=0, mode="promise_in_bounds")
    nsmall = jnp.take_along_axis(small, mate, axis=0, mode="promise_in_bounds")
    thr = jnp.maximum(jnp.minimum(big, nbig), jnp.maximum(small, nsmall))
    return u & (jnp.where(lo < thr, 0, 0xFFFF) | jnp.where(hi < thr, 0, -65536))


def _prune_rows(w_bf16):
    u = pltpu.bitcast(w_bf16, I32)
    return [_prune_packed(u[8 * i:8 * i + 8]) for i in range(u.shape[0] // 8)]


def _lhs(a11, a12, a21, a22):
    return [a11 + a22, a21 + a22, a11, a22, a11 + a12, a21 - a11, a12 - a22]


_RHS = [(0, 3), (0, None), (1, 3), (2, 0), (3, None), (1, 0), (2, 3)]


def _rhs(*b):
    return [b[p] if q is None else b[p] - b[q] for p, q in _RHS]


_T_OF_P = {1: 1, 2: 3, 3: 2, 4: 4}
_SHARED = {"P0": {0: 1, 3: -1}, "P1": {2: 1, 3: 1}, "P2": {1: 1, 3: 1}, "P3": {0: 1, 2: 1},
           "P4": {0: 1, 1: 1}, "Q0": {1: 1, 2: -1}}
_LAST = {"P5": 3, "P6": 0, "Q1": 2, "Q2": 1}
_BIAS = {("P4", 4): 0, ("P4", 1): 1, ("P1", 4): 2, ("P1", 1): 3}
N_WEIGHTS = 51


def _passes():
    def p0(j):
        return [("P0", (j, n), n, "T%d" % j) for n in (2, 0, 1)]

    def p(c):
        return [("P%d" % c, n, 7 * c - 4 + n, "P%d" % c) for n in range(7)]

    def q(c, blk):
        return [("Q%d" % c, blk, 45 + 2 * c + (blk >> 1), "Q%d%d" % (c, blk & 1))]

    return (p0(0) + q(0, 0) + p0(1) + q(0, 2) + p(3) + q(0, 1) + p(1) + q(0, 3)
            + p(4) + q(1, 0) + p(2) + q(1, 2) + p(6) + q(1, 1) + p(5) + q(1, 3)
            + q(2, 0) + q(2, 2) + q(2, 1) + q(2, 3))


PASSES = _passes()
STEP_CYCLES = len(PASSES) // 4 * H
PREP_SPAN, PREP_LEAD = 250, 30


def _prepare_weights(wbuf, bbuf, wt_ref, bias_ref, arrive):
    def transposed(parts):
        return pltpu.bitcast(jnp.concatenate(parts, axis=0), BF16).T.astype(F32)

    kt = []
    for i in range(4):
        arrive(i)
        kt.append(transposed(_prune_rows(wbuf[128 * i:128 * (i + 1), :])))
    tail = _prune_rows(wbuf[512:D, :])
    kt.append(transposed(tail + tail))
    low = lax.broadcasted_iota(I32, (H, 128), 1) < 64

    def quarter(t, i):
        return kt[t][H * i:H * (i + 1)]

    def put(n, v):
        wt_ref[n] = pltpu.bitcast(v.astype(BF16), I32)

    ab, cd = [[_lhs(quarter(t, i), quarter(t + 1, i), quarter(t, i + 2), quarter(t + 1, i + 2))
               for i in range(2)] for t in (0, 2)]
    put(0, jnp.where(low, ab[0][0] - ab[1][0], ab[0][0]))
    put(1, jnp.where(low, cd[1][0] - cd[0][0], ab[1][0]))
    put(2, jnp.concatenate([ab[1][0][:, :64], cd[0][0][:, :64]], axis=1))
    for c in range(1, 7):
        blocks = []
        for i in range(2):
            if c >= 5:
                mixed = jnp.where(low, cd[i][c], quarter(4, i + 2 if c == 5 else i))
            elif _T_OF_P[c] == c:
                mixed = cd[i][c]
            else:
                mixed = jnp.where(low, cd[i][c], cd[i][_T_OF_P[c]])
            blocks += [ab[i][c], mixed]
        for n, v in enumerate(_lhs(*blocks)):
            put(7 * c - 4 + n, v)
    for i in range(2):
        put(45 + i, jnp.where(low, 0.0, cd[i][0]))
        put(47 + i, jnp.where(low, quarter(4, i + 2), cd[i][5]))
        put(49 + i, jnp.where(low, quarter(4, i), cd[i][6]))
    bias = bbuf[...].reshape(1, D).astype(F32)
    bias_ref[...] = jnp.broadcast_to(bias, (128, D)).T


def _operand_slabs(load, name):
    rows = range(64 - SLAB, -1, -SLAB)

    def level1(which, u1, u2, j1, j2, k):
        src = [(u1, j1), (u1, j2), (u2, j1), (u2, j2)]
        p, q = _RHS[which]
        v = load(*src[p], k)
        return v if q is None else v - load(*src[q], k)

    def s_rhs(which, u, j, k):
        return level1(which, *((0, 2), (1, 3), (4, 6))[u], j, j + 2, k)

    def t_rhs(which, j, k):
        return level1(which, 5, 7, j + 2, j, k)

    c = int(name[1])
    if name[0] == "T":
        return [functools.partial(s_rhs, 0, u, c, k) for u in (2, 1, 0) for k in rows]
    if name[0] == "Q":
        j = int(name[2])

        def bottom(k):
            return [t_rhs(4 + c if c else 0, j, k)]

        def top(k):
            return [load(8, j + 2 * (c - 1), k) if c else jnp.zeros((SLAB, 128), F32)]
    else:
        def fourth(j, k):
            return t_rhs(_T_OF_P[c], j, k) if c < 5 else load(8, j + 2 if c == 5 else j, k)

        def bottom(k):
            return _rhs(s_rhs(c, 1, 0, k), s_rhs(c, 1, 1, k), fourth(0, k), fourth(1, k))

        def top(k):
            return _rhs(*[s_rhs(c, u, j, k) for u in (0, 2) for j in range(2)])
    return [functools.partial(fn, k) for fn in (bottom, top) for k in rows]


def _operands(name, slabs):
    def cat(parts):
        return jnp.concatenate(parts, axis=0).astype(BF16)

    slabs = slabs[::-1]
    if name[0] == "T":
        a, b, c = slabs[0:4], slabs[4:8], slabs[8:12]
        return {2: cat(a + c), 0: cat(a + b), 1: cat(c + b)}
    return [cat([v[n] for v in slabs]) for n in range(len(slabs[0]))]


def _gemm(steps, load, store, weights, bias_ref, events):
    slabs = {}
    events = list(events)
    for s in range(steps):
        for p, (_, _, _, name) in enumerate(PASSES):
            if (s, name) not in slabs:
                slabs[s, name] = []
                thunks = _operand_slabs(functools.partial(load, s), name)
                start = s * STEP_CYCLES + p // 4 * H - PREP_LEAD - PREP_SPAN
                for i, thunk in enumerate(thunks):
                    events.append((start + PREP_SPAN * i / (len(thunks) - 1),
                                   lambda out=slabs[s, name], fn=thunk: out.append(fn())))
    events.sort(key=lambda e: e[0])

    for s in range(steps):
        shared, rhs, m = {}, {}, {}

        def add_shared(out, blk, acc=None):
            terms = [(signs[out], shared[cls, blk]) for cls, signs in _SHARED.items() if out in signs]
            for sign, v in sorted(terms, key=lambda t: -t[0]):
                acc = v if acc is None else acc + v if sign > 0 else acc - v
            return acc

        def put(cls, blk, v):
            if cls in _SHARED:
                shared[cls, blk] = v
            else:
                out = _LAST[cls]
                store(s, 2 * (out >> 1) + (blk >> 1), 2 * (out & 1) + (blk & 1), v)

        for p, (cls, n, block, name) in enumerate(PASSES):
            while events and events[0][0] < s * STEP_CYCLES + (p // 4 + 1) * H:
                events.pop(0)[1]()
            if name not in rhs:
                rhs[name] = _operands(name, slabs[s, name])

            def dot(operand):
                return jnp.dot(weights(s, p, block), rhs[name][operand], preferred_element_type=F32)

            if cls == "P0":
                if block == 2:
                    m[0] = dot(block)
                else:
                    put(cls, 2 * block + n[0], m[0] + dot(block))
            elif cls == "Q0":
                put(cls, n, dot(0))
            elif cls[0] == "Q":
                put(cls, n, add_shared(_LAST[cls], n) + dot(0))
            elif n < 5:
                if (cls, n) in _BIAS:
                    m[n] = bias_ref[pl.ds(H * _BIAS[cls, n], H), :] + dot(n)
                else:
                    m[n] = dot(n)
                if n == 3:
                    part = [m[0] + m[3], m[2], m[1] + m[3], (m[1] - m[0]) + m[2]]
                    if cls in _LAST:
                        part = [add_shared(_LAST[cls], blk, part[blk]) for blk in range(4)]
                    put(cls, 2, part[2])
                elif n == 4:
                    put(cls, 1, part[1] + m[4])
            elif n == 5:
                put(cls, 3, part[3] + dot(n))
            else:
                put(cls, 0, part[0] + m[4] + dot(n))
    for _, thunk in events:
        thunk()


UNITS = 16
RING = 5
GROUPS = 24
READS = 12
WRITES = 8
WRITE_AT = 450
WAIT_LEAD = 300
TAIL = 5
READ_ORDER, READ_ORDER_FIRST = "s0 r3 r1 r0 r2", "r3 r1 r0 r2 s0"
WRITE_ORDER, WRITE_ORDER_LAST = "s0 r0 r1 r2 r3", "r1 r3 r2 r0 s0"


def _position(order, q):
    pos = {"s": 0, "r": 0}
    for i, (axis, bit) in enumerate(order.split()):
        pos[axis] |= ((q >> i) & 1) << int(bit)
    return pos["s"], pos["r"]


def _kernel(x_hbm, w_hbm, b_hbm, o_hbm, xbuf, obuf, wbuf, bbuf, wt_ref, bias_ref, sems):
    def ring(u):
        return jnp.where(u >= 2 * RING, u - 2 * RING, jnp.where(u >= RING, u - RING, u))

    def read(j, sem, band=slice(None), col=0, n=1024):
        r = ring(j >> 1)
        src = pl.multiple_of((j & 3) * 1024 + col, 512)
        dst = pl.multiple_of((r & 1) * 2048 + (j & 1) * 1024 + col, 512)
        return pltpu.make_async_copy(x_hbm.at[j >> 2, :, band, :, pl.ds(src, n)],
                                     xbuf.at[r >> 1, :, band, :, pl.ds(dst, n)], sems.at[sem])

    def first_read(k):
        rows = (pl.ds(0, 5), pl.ds(5, 4), slice(None))[min(k, 2)]
        where = (0, rows, slice(None), slice(None), pl.ds(max(k - 1, 0) * 512, 512))
        return pltpu.make_async_copy(x_hbm.at[where], xbuf.at[where], sems.at[k % 4])

    def write(u, q, order=WRITE_ORDER):
        s, band = _position(order, q)
        dst = pl.multiple_of((u & 1) * 2048 + s * 1024, 1024)
        return pltpu.make_async_copy(obuf.at[u, :, band, :, pl.ds(s * 1024, 1024)],
                                     o_hbm.at[u >> 1, :, band, :, pl.ds(dst, 1024)], sems.at[3])

    def late_read(pair, *where, sem=4):
        return pltpu.make_async_copy(
            x_hbm.at[(pair, *where)], xbuf.at[(pair - 3, *where)], sems.at[sem])

    w_head = pltpu.make_async_copy(w_hbm.at[pl.ds(0, 128)], wbuf.at[pl.ds(0, 128)], sems.at[3])
    w_rest = [pltpu.make_async_copy(
                  w_hbm.at[pl.ds(128, D - 128)], wbuf.at[pl.ds(128, D - 128)], sems.at[4]),
              pltpu.make_async_copy(b_hbm, bbuf, sems.at[4])]
    late = [late_read(6), late_read(7, pl.ds(0, 8)), late_read(7, 8, pl.ds(0, 16 - TAIL))]
    late_tail = late_read(7, 8, pl.ds(16 - TAIL, TAIL), sem=5)
    for copy in [w_head] + w_rest + [first_read(0), first_read(1)]:
        copy.start(priority=1)

    def arrive(i):
        if i == 0:
            w_head.wait()
        if i == 1:
            for copy in w_rest:
                copy.wait()
            for copy in late + [late_tail]:
                copy.start(priority=1)

    _prepare_weights(wbuf, bbuf, wt_ref, bias_ref, arrive)

    pins = [divmod(e * STEP_CYCLES // SLAB // READS, H // SLAB) for e in range(READS)]
    pin_ref = xbuf.at[2, 0]
    for e, (rnd, k) in enumerate(pins):
        v = pltpu.bitcast(wt_ref[PASSES[4 * rnd][2], pl.ds(8 * k, 8), :], BF16)
        pin_ref[0, :, pl.ds(2048 + 128 * e, 128)] = v[:8]
        pin_ref[1, :, pl.ds(2048 + 128 * e, 128)] = v[8:]

    def unit(u, carry):
        r = jnp.where(u >= GROUPS // 2, u - GROUPS // 2 + 6, ring(u))
        x_ref = xbuf.at[r >> 1, :, :, :, pl.ds(pl.multiple_of((r & 1) * 2048, 2048), 2048)]
        events, spans, pinned = [], {}, {}

        def during(lo, hi):
            if (lo, hi) not in spans:
                spans[lo, hi] = (u == lo if hi == lo + 1 else u < hi if lo == 0
                                 else u >= lo if hi == UNITS else (u >= lo) & (u < hi))
            return pl.when(spans[lo, hi])

        def group(k):
            return jnp.minimum(3 * u + 1 + k, GROUPS - 1), (GROUPS - 2 - k) // 3 + 1

        def wait_group(k, first):
            j, end = group(k)
            during(first, end)(read(j, k % 3).wait)

        def start_read(i):
            q = i - 16
            j, end = group(q >> 5)
            s, band = _position(READ_ORDER, q & 31)
            sem = jnp.where(u == 0, 3, 0) if 0 <= q < 16 else (q >> 5) % 3
            if q < 32:
                s0, band0 = _position(READ_ORDER_FIRST, q & 31)
                s, band = jnp.where(u == 0, s0, s), jnp.where(u == 0, band0, band)
            during(0, end)(read(j, sem, band, s * 512, 512).start)
            rnd, k = pins[i % READS]
            v = pin_ref[pl.ds(0, 2), :, pl.ds(2048 + 128 * (i % READS), 128)].reshape(SLAB, 128)
            pinned[i // READS, 4 * rnd, k] = pltpu.bitcast(v, I32)

        def start_write(q):
            copy = write(jnp.clip(2 * u - 16 + (q >> 5), 0, UNITS - 1), q & 31)
            during(*((8, 16), (8, 15), (7, 14))[q >> 5])(copy.start)

        def start_last_write(*args):
            during(15, 16)(write(*args).start)

        def at(step, cycle, fn, *args):
            events.append((step * STEP_CYCLES + cycle, functools.partial(fn, *args)))

        at(5, -WAIT_LEAD, wait_group, 0, 1)
        at(8, -WAIT_LEAD - 20, wait_group, 1, 0)
        at(3, -WAIT_LEAD, wait_group, -1, 1)
        for k, step in enumerate((0, 1, 2, 4, 5)):
            at(step, -WAIT_LEAD, lambda k: during(0, 1)(first_read(k).wait), k)
        at(7, WRITE_AT - 1, lambda: during(7, 8)(lambda: [c.wait() for c in late] and None))
        at(8, -WAIT_LEAD, lambda: during(7, 8)(late_tail.wait))
        for i in range(8 * WRITES):
            at(i // WRITES, WRITE_AT, start_write, i + WRITES)
            if i < WRITES:
                at(0, WRITE_AT - 1, start_last_write, jnp.int32(14), i)
            if 32 <= i < 48:
                at(i // WRITES, WRITE_AT, start_last_write, jnp.int32(15), i - 32, WRITE_ORDER_LAST)
        for i in range(8 * READS):
            rnd, k = pins[i % READS]
            at(i // READS, rnd * H + SLAB * k, start_read, i)

        def weights(s, p, block):
            slabs = range(H // SLAB)
            if not any((s, p, k) in pinned for k in slabs):
                return pltpu.bitcast(wt_ref[block], BF16)
            parts = [pinned[s, p, k] if (s, p, k) in pinned else wt_ref[block, pl.ds(8 * k, 8), :]
                     for k in slabs]
            return pltpu.bitcast(jnp.concatenate(parts, axis=0), BF16)

        def load(s, xunit, tile, row):
            band = (s & 1) * 72 + xunit * 8 + row // 8
            cols = pl.ds((s >> 1) * 512 + tile * 128, 128)
            v = x_ref[band // 16, pl.ds(band % 16, SLAB // 8), :, cols]
            return v.astype(F32).reshape(SLAB, 128)

        def store(s, quarter, tile, v):
            cols = pl.ds((s >> 1) * 512 + tile * 128, 128)
            for k in range(H // 8):
                band = (s & 1) * 72 + quarter * (H // 8) + k
                obuf[u, band // 16, band % 16, :, cols] = v[8 * k:8 * k + 8].astype(BF16)

        _gemm(8, load, store, weights, bias_ref, events)
        return carry

    lax.fori_loop(0, UNITS, unit, 0)
    for q in range(16, 32):
        write(jnp.int32(15), q, WRITE_ORDER_LAST).start()
    pltpu.make_async_copy(o_hbm, o_hbm, sems.at[3]).wait()


@jax.jit
def pallas_standalone__structured_sparse_n_m__ragged_kernel(
    x: jax.Array,
    w: jax.Array,
    b: jax.Array,
):
    B, S, _ = x.shape
    assert x.shape == (UNITS, 4096, D) and w.shape == (D, D)
    view = (B // 2, 9, 16, 8, S)
    out = pl.pallas_call(
        _kernel,
        in_specs=[pl.BlockSpec(memory_space=pl.ANY)] * 3,
        out_specs=pl.BlockSpec(memory_space=pl.ANY),
        out_shape=jax.ShapeDtypeStruct(view, x.dtype),
        scratch_shapes=[
            pltpu.VMEM((5, 9, 16, 8, S), x.dtype),
            pltpu.VMEM((UNITS, 9, 16, 8, S // 2), x.dtype),
            pltpu.VMEM((D, D), w.dtype),
            pltpu.VMEM((D,), b.dtype),
            pltpu.VMEM((N_WEIGHTS, H // 2, 128), I32),
            pltpu.VMEM((D, 128), F32),
            pltpu.SemaphoreType.DMA((6,)),
        ],
        compiler_params=pltpu.CompilerParams(
            vmem_limit_bytes=127 * 1024 * 1024,
            disable_bounds_checks=True,
            flags={"XLA_TPU_RESCHEDULE_DMA_DONES": True},
        ),
    )(jnp.transpose(x, (0, 2, 1)).reshape(view), w, b)
    return jnp.transpose(out.reshape(B, D, S), (0, 2, 1))
```

```python
import functools

import jax
import jax.numpy as jnp
from jax import lax
import jax.experimental.pallas as pl
import jax.experimental.pallas.tpu as pltpu

F32, BF16, I32 = jnp.float32, jnp.bfloat16, jnp.int32

D = 576
H = D // 4
SLAB = 16


def _prune_packed(u):
    mate = lax.broadcasted_iota(I32, u.shape, 0) ^ 1
    lo = pltpu.bitcast((u << 16) & 0x7FFFFFFF, F32)
    hi = pltpu.bitcast(u & 0x7FFF0000, F32)
    big, small = jnp.maximum(lo, hi), jnp.minimum(lo, hi)
    nbig = jnp.take_along_axis(big, mate, axis=0, mode="promise_in_bounds")
    nsmall = jnp.take_along_axis(small, mate, axis=0, mode="promise_in_bounds")
    thr = jnp.maximum(jnp.minimum(big, nbig), jnp.maximum(small, nsmall))
    return u & (jnp.where(lo < thr, 0, 0xFFFF) | jnp.where(hi < thr, 0, -65536))


def _prune_rows(w_bf16):
    u = pltpu.bitcast(w_bf16, I32)
    return [_prune_packed(u[8 * i:8 * i + 8]) for i in range(u.shape[0] // 8)]


def _lhs(a11, a12, a21, a22):
    return [a11 + a22, a21 + a22, a11, a22, a11 + a12, a21 - a11, a12 - a22]


_RHS = [(0, 3), (0, None), (1, 3), (2, 0), (3, None), (1, 0), (2, 3)]


def _rhs(*b):
    return [b[p] if q is None else b[p] - b[q] for p, q in _RHS]


_T_OF_P = {1: 1, 2: 3, 3: 2, 4: 4}
_SHARED = {"P0": {0: 1, 3: -1}, "P1": {2: 1, 3: 1}, "P2": {1: 1, 3: 1}, "P3": {0: 1, 2: 1},
           "P4": {0: 1, 1: 1}, "Q0": {1: 1, 2: -1}}
_LAST = {"P5": 3, "P6": 0, "Q1": 2, "Q2": 1}
_BIAS = {("P4", 4): 0, ("P4", 1): 1, ("P1", 4): 2, ("P1", 1): 3}
N_WEIGHTS = 51


def _passes():
    def p0(j):
        return [("P0", (j, n), n, "T%d" % j) for n in (2, 0, 1)]

    def p(c):
        return [("P%d" % c, n, 7 * c - 4 + n, "P%d" % c) for n in range(7)]

    def q(c, blk):
        return [("Q%d" % c, blk, 45 + 2 * c + (blk >> 1), "Q%d%d" % (c, blk & 1))]

    return (p0(0) + q(0, 0) + p0(1) + q(0, 2) + p(3) + q(0, 1) + p(1) + q(0, 3)
            + p(4) + q(1, 0) + p(2) + q(1, 2) + p(6) + q(1, 1) + p(5) + q(1, 3)
            + q(2, 0) + q(2, 2) + q(2, 1) + q(2, 3))


PASSES = _passes()
STEP_CYCLES = len(PASSES) // 4 * H
PREP_SPAN, PREP_LEAD = 250, 30


def _prepare_weights(wbuf, bbuf, wt_ref, bias_ref, arrive):
    def transposed(parts):
        return pltpu.bitcast(jnp.concatenate(parts, axis=0), BF16).T.astype(F32)

    kt = []
    for i in range(4):
        arrive(i)
        kt.append(transposed(_prune_rows(wbuf[128 * i:128 * (i + 1), :])))
    tail = _prune_rows(wbuf[512:D, :])
    kt.append(transposed(tail + tail))
    low = lax.broadcasted_iota(I32, (H, 128), 1) < 64

    def quarter(t, i):
        return kt[t][H * i:H * (i + 1)]

    def put(n, v):
        wt_ref[n] = pltpu.bitcast(v.astype(BF16), I32)

    ab, cd = [[_lhs(quarter(t, i), quarter(t + 1, i), quarter(t, i + 2), quarter(t + 1, i + 2))
               for i in range(2)] for t in (0, 2)]
    put(0, jnp.where(low, ab[0][0] - ab[1][0], ab[0][0]))
    put(1, jnp.where(low, cd[1][0] - cd[0][0], ab[1][0]))
    put(2, jnp.concatenate([ab[1][0][:, :64], cd[0][0][:, :64]], axis=1))
    for c in range(1, 7):
        blocks = []
        for i in range(2):
            if c >= 5:
                mixed = jnp.where(low, cd[i][c], quarter(4, i + 2 if c == 5 else i))
            elif _T_OF_P[c] == c:
                mixed = cd[i][c]
            else:
                mixed = jnp.where(low, cd[i][c], cd[i][_T_OF_P[c]])
            blocks += [ab[i][c], mixed]
        for n, v in enumerate(_lhs(*blocks)):
            put(7 * c - 4 + n, v)
    for i in range(2):
        put(45 + i, jnp.where(low, 0.0, cd[i][0]))
        put(47 + i, jnp.where(low, quarter(4, i + 2), cd[i][5]))
        put(49 + i, jnp.where(low, quarter(4, i), cd[i][6]))
    bias = bbuf[...].reshape(1, D).astype(F32)
    bias_ref[...] = jnp.broadcast_to(bias, (128, D)).T


def _operand_slabs(load, name):
    rows = range(64 - SLAB, -1, -SLAB)

    def level1(which, u1, u2, j1, j2, k):
        src = [(u1, j1), (u1, j2), (u2, j1), (u2, j2)]
        p, q = _RHS[which]
        v = load(*src[p], k)
        return v if q is None else v - load(*src[q], k)

    def s_rhs(which, u, j, k):
        return level1(which, *((0, 2), (1, 3), (4, 6))[u], j, j + 2, k)

    def t_rhs(which, j, k):
        return level1(which, 5, 7, j + 2, j, k)

    c = int(name[1])
    if name[0] == "T":
        return [functools.partial(s_rhs, 0, u, c, k) for u in (2, 1, 0) for k in rows]
    if name[0] == "Q":
        j = int(name[2])

        def bottom(k):
            return [t_rhs(4 + c if c else 0, j, k)]

        def top(k):
            return [load(8, j + 2 * (c - 1), k) if c else jnp.zeros((SLAB, 128), F32)]
    else:
        def fourth(j, k):
            return t_rhs(_T_OF_P[c], j, k) if c < 5 else load(8, j + 2 if c == 5 else j, k)

        def bottom(k):
            return _rhs(s_rhs(c, 1, 0, k), s_rhs(c, 1, 1, k), fourth(0, k), fourth(1, k))

        def top(k):
            return _rhs(*[s_rhs(c, u, j, k) for u in (0, 2) for j in range(2)])
    return [functools.partial(fn, k) for fn in (bottom, top) for k in rows]


def _operands(name, slabs):
    def cat(parts):
        return jnp.concatenate(parts, axis=0).astype(BF16)

    slabs = slabs[::-1]
    if name[0] == "T":
        a, b, c = slabs[0:4], slabs[4:8], slabs[8:12]
        return {2: cat(a + c), 0: cat(a + b), 1: cat(c + b)}
    return [cat([v[n] for v in slabs]) for n in range(len(slabs[0]))]


def _gemm(steps, load, store, weights, bias_ref, events):
    slabs = {}
    events = list(events)
    for s in range(steps):
        for p, (_, _, _, name) in enumerate(PASSES):
            if (s, name) not in slabs:
                slabs[s, name] = []
                thunks = _operand_slabs(functools.partial(load, s), name)
                start = s * STEP_CYCLES + p // 4 * H - PREP_LEAD - PREP_SPAN
                for i, thunk in enumerate(thunks):
                    events.append((start + PREP_SPAN * i / (len(thunks) - 1),
                                   lambda out=slabs[s, name], fn=thunk: out.append(fn())))
    events.sort(key=lambda e: e[0])

    for s in range(steps):
        shared, rhs, m = {}, {}, {}

        def add_shared(out, blk, acc=None):
            terms = [(signs[out], shared[cls, blk]) for cls, signs in _SHARED.items() if out in signs]
            for sign, v in sorted(terms, key=lambda t: -t[0]):
                acc = v if acc is None else acc + v if sign > 0 else acc - v
            return acc

        def put(cls, blk, v):
            if cls in _SHARED:
                shared[cls, blk] = v
            else:
                out = _LAST[cls]
                store(s, 2 * (out >> 1) + (blk >> 1), 2 * (out & 1) + (blk & 1), v)

        for p, (cls, n, block, name) in enumerate(PASSES):
            while events and events[0][0] < s * STEP_CYCLES + (p // 4 + 1) * H:
                events.pop(0)[1]()
            if name not in rhs:
                rhs[name] = _operands(name, slabs[s, name])

            def dot(operand):
                return jnp.dot(weights(s, p, block), rhs[name][operand], preferred_element_type=F32)

            if cls == "P0":
                if block == 2:
                    m[0] = dot(block)
                else:
                    put(cls, 2 * block + n[0], m[0] + dot(block))
            elif cls == "Q0":
                put(cls, n, dot(0))
            elif cls[0] == "Q":
                put(cls, n, add_shared(_LAST[cls], n) + dot(0))
            elif n < 5:
                if (cls, n) in _BIAS:
                    m[n] = bias_ref[pl.ds(H * _BIAS[cls, n], H), :] + dot(n)
                else:
                    m[n] = dot(n)
                if n == 3:
                    part = [m[0] + m[3], m[2], m[1] + m[3], (m[1] - m[0]) + m[2]]
                    if cls in _LAST:
                        part = [add_shared(_LAST[cls], blk, part[blk]) for blk in range(4)]
                    put(cls, 2, part[2])
                elif n == 4:
                    put(cls, 1, part[1] + m[4])
            elif n == 5:
                put(cls, 3, part[3] + dot(n))
            else:
                put(cls, 0, part[0] + m[4] + dot(n))
    for _, thunk in events:
        thunk()


UNITS = 16
GROUPS = 24
READS = 12
WRITES = 8
WRITE_AT = 300
WAIT_LEAD = 300
TAIL = 6
READ_ORDER, WRITE_ORDER = "s0 r1 r2 r3 r0", "s0 r0 r1 r2 r3"
TOKEN_ORDER = "r1 r2 r3 r0 s0"


def _position(order, q):
    pos = {"s": 0, "r": 0}
    for i, (axis, bit) in enumerate(order.split()):
        pos[axis] |= ((q >> i) & 1) << int(bit)
    return pos["s"], pos["r"]


def _stream(x_hbm, w_hbm, b_hbm, o_hbm, xbuf, obuf, wbuf, bbuf, wt_ref, bias_ref, sems):
    def slot(pair):
        return pl.ds(9 * jnp.where(pair >= 3, pair - 3, pair), 9)

    def read(pair, band, col, n, sem):
        cols = pl.ds(pl.multiple_of(col, 512), n)
        return pltpu.make_async_copy(
            x_hbm.at[pair, :, band, :, cols], xbuf.at[slot(pair), band, :, cols], sems.at[sem])

    def first_read(k):
        rows = (pl.ds(0, 5), pl.ds(5, 4), pl.ds(0, 9))[min(k, 2)]
        where = (rows, slice(None), slice(None), pl.ds(max(k - 1, 0) * 512, 512))
        return pltpu.make_async_copy(x_hbm.at[(0, *where)], xbuf.at[where], sems.at[k % 4])

    def late_read(pair, a, n, band=slice(None), sem=4):
        return pltpu.make_async_copy(x_hbm.at[pair, pl.ds(a, n), band],
                                     xbuf.at[pl.ds(9 * (pair - 3) + a, n), band], sems.at[sem])

    def write(u, order, q):
        s, band = _position(order, q)
        dst = pl.multiple_of((u & 1) * 2048 + s * 1024, 1024)
        return pltpu.make_async_copy(obuf.at[u, :, band, :, pl.ds(s * 1024, 1024)],
                                     o_hbm.at[u >> 1, :, band, :, pl.ds(dst, 1024)], sems.at[3])

    w_head = pltpu.make_async_copy(w_hbm.at[pl.ds(0, 128)], wbuf.at[pl.ds(0, 128)], sems.at[3])
    w_rest = [pltpu.make_async_copy(
                  w_hbm.at[pl.ds(128, D - 128)], wbuf.at[pl.ds(128, D - 128)], sems.at[4]),
              pltpu.make_async_copy(b_hbm, bbuf, sems.at[4])]
    late = [late_read(6, 0, 9), late_read(7, 0, 8), late_read(7, 8, 1, pl.ds(0, 16 - TAIL))]
    late_tail = late_read(7, 8, 1, pl.ds(16 - TAIL, TAIL), sem=5)
    for copy in [w_head] + w_rest + [first_read(0), first_read(1)]:
        copy.start(priority=1)

    def arrive(i):
        if i == 0:
            w_head.wait()
        if i == 1:
            for copy in w_rest:
                copy.wait()
            for copy in late + [late_tail]:
                copy.start(priority=1)

    _prepare_weights(wbuf, bbuf, wt_ref, bias_ref, arrive)

    pins = [divmod(e * STEP_CYCLES // SLAB // READS, H // SLAB) for e in range(READS)]
    pin_ref = xbuf.at[45]
    for e, (rnd, k) in enumerate(pins):
        v = pltpu.bitcast(wt_ref[PASSES[4 * rnd][2], pl.ds(8 * k, 8), :], BF16)
        pin_ref[0, :, pl.ds(128 * e, 128)] = v[:8]
        pin_ref[1, :, pl.ds(128 * e, 128)] = v[8:]

    def unit(u, carry):
        x_ref = xbuf.at[slot(u >> 1), :, :, pl.ds(pl.multiple_of((u & 1) * 2048, 2048), 2048)]
        events, spans, pinned = [], {}, {}

        def during(lo, hi):
            if (lo, hi) not in spans:
                spans[lo, hi] = (u == lo if hi == lo + 1 else u < hi if lo == 0
                                 else u >= lo if hi == UNITS else (u >= lo) & (u < hi))
            return pl.when(spans[lo, hi])

        def group(k):
            return jnp.minimum(3 * u + 1 + k, GROUPS - 1), (GROUPS - 2 - k) // 3 + 1

        def wait_group(k, first):
            j, end = group(k)
            during(first, end)(read(j >> 2, slice(None), (j & 3) * 1024, 1024, k % 3).wait)

        def wait_first(k):
            during(0, 1)(first_read(k).wait)

        def wait_late(copies):
            for copy in copies:
                during(7, 8)(copy.wait)

        def start_read(i):
            q = i - 16
            j, end = group(q >> 5)
            s, band = _position(READ_ORDER, q & 31)
            sem = jnp.where(u == 0, 3, 0) if 0 <= q < 16 else (q >> 5) % 3
            if q < 32:
                s0, band0 = _position(TOKEN_ORDER, q & 31)
                s, band = jnp.where(u == 0, s0, s), jnp.where(u == 0, band0, band)
            during(0, end)(read(j >> 2, band, (s + 2 * (j & 3)) * 512, 512, sem).start)
            rnd, k = pins[i % READS]
            v = pin_ref[pl.ds(0, 2), :, pl.ds(128 * (i % READS), 128)].reshape(SLAB, 128)
            pinned[i // READS, 4 * rnd, k] = pltpu.bitcast(v, I32)

        def start_write(q):
            copy = write(jnp.clip(2 * u - 16 + (q >> 5), 0, UNITS - 1), WRITE_ORDER, q & 31)
            during(*((8, 16), (8, 15), (7, 14))[q >> 5])(copy.start)

        def start_last_write(v, order, q):
            during(15, 16)(write(jnp.int32(v), order, q).start)

        def at(step, cycle, fn, *args):
            events.append((step * STEP_CYCLES + cycle, functools.partial(fn, *args)))

        at(5, -WAIT_LEAD, wait_group, 0, 1)
        at(8, -WAIT_LEAD - 20, wait_group, 1, 0)
        at(3, -WAIT_LEAD, wait_group, -1, 1)
        for k, step in enumerate((0, 1, 2, 4, 5)):
            at(step, -WAIT_LEAD, wait_first, k)
        at(7, WRITE_AT - 1, wait_late, late)
        at(8, -10, wait_late, [late_tail])
        for i in range(8 * WRITES):
            step = i // WRITES
            at(step, WRITE_AT if step else 50, start_write, i + WRITES)
            if step == 0:
                at(step, 49, start_last_write, 14, WRITE_ORDER, i)
            if step in (4, 5):
                at(step, WRITE_AT, start_last_write, 15, TOKEN_ORDER, i - 32)
        for i in range(8 * READS):
            rnd, k = pins[i % READS]
            at(i // READS, rnd * H + SLAB * k, start_read, i)

        def weights(s, p, block):
            slabs = range(H // SLAB)
            if not any((s, p, k) in pinned for k in slabs):
                return pltpu.bitcast(wt_ref[block], BF16)
            parts = [pinned[s, p, k] if (s, p, k) in pinned else wt_ref[block, pl.ds(8 * k, 8), :]
                     for k in slabs]
            return pltpu.bitcast(jnp.concatenate(parts, axis=0), BF16)

        def load(s, xunit, tile, row):
            band = (s & 1) * 72 + xunit * 8 + row // 8
            cols = pl.ds((s >> 1) * 512 + tile * 128, 128)
            v = x_ref[band // 16, pl.ds(band % 16, SLAB // 8), :, cols]
            return v.astype(F32).reshape(SLAB, 128)

        def store(s, quarter, tile, v):
            cols = pl.ds((s >> 1) * 512 + tile * 128, 128)
            for k in range(H // 8):
                band = (s & 1) * 72 + quarter * (H // 8) + k
                obuf[u, band // 16, band % 16, :, cols] = v[8 * k:8 * k + 8].astype(BF16)

        _gemm(8, load, store, weights, bias_ref, events)
        return carry

    lax.fori_loop(0, UNITS, unit, 0)
    for q in range(16, 32):
        write(jnp.int32(15), TOKEN_ORDER, q).start()
    pltpu.make_async_copy(o_hbm, o_hbm, sems.at[3]).wait()


def _kernel(*refs):
    pl.run_scoped(functools.partial(_stream, *refs), pltpu.SemaphoreType.DMA((6,)))


@jax.jit
def pallas_standalone__structured_sparse_n_m__ragged_kernel(
    x: jax.Array,
    w: jax.Array,
    b: jax.Array,
):
    B, S, _ = x.shape
    assert x.shape == (UNITS, 4096, D) and w.shape == (D, D)
    view = (B // 2, 9, 16, 8, S)
    out = pl.pallas_call(
        _kernel,
        in_specs=[pl.BlockSpec(memory_space=pl.ANY)] * 3,
        out_specs=pl.BlockSpec(memory_space=pl.ANY),
        out_shape=jax.ShapeDtypeStruct(view, x.dtype),
        scratch_shapes=[
            pltpu.VMEM((5 * 9 + 1, 16, 8, S), x.dtype),
            pltpu.VMEM((UNITS, 9, 16, 8, S // 2), x.dtype),
            pltpu.VMEM((D, D), w.dtype),
            pltpu.VMEM((D,), b.dtype),
            pltpu.VMEM((N_WEIGHTS, H // 2, 128), I32),
            pltpu.VMEM((D, 128), F32),
        ],
        compiler_params=pltpu.CompilerParams(
            vmem_limit_bytes=127 * 1024 * 1024,
            disable_bounds_checks=True,
            flags={"XLA_TPU_RESCHEDULE_DMA_DONES": True},
        ),
    )(jnp.transpose(x, (0, 2, 1)).reshape(view), w, b)
    return jnp.transpose(out.reshape(B, D, S), (0, 2, 1))
```
